```python
import jax
import jax.numpy as jnp

def _softmax(x, axis=-1):
    return jax.nn.softmax(x, axis=axis)
def _gelu(x):
    return jax.nn.gelu(x, approximate=True)
def _silu(x):
    return jax.nn.silu(x)
def _sigmoid(x):
    return jax.nn.sigmoid(x)
def _layernorm(x, axis=-1, eps=1e-5):
    m = jnp.mean(x, axis=axis, keepdims=True)
    v = jnp.var(x, axis=axis, keepdims=True)
    return (x - m) / jnp.sqrt(v + eps)
def _scatter_add(tgt, idx, src, axis=0):
    return tgt.at[idx].add(src)
def _segment_sum(src, seg, n):
    return jax.ops.segment_sum(src, seg, n)
class _Rng:
    def __init__(self, key):
        self._k = key
    def _next(self):
        self._k, sub = jax.random.split(self._k)
        return sub
    def normal(self, shape):
        return jax.random.normal(self._next(), shape, dtype=jnp.bfloat16)
    def randint(self, lo, hi, shape):
        return jax.random.randint(self._next(), shape, lo, hi, dtype=jnp.int32)
    def uniform(self, shape, lo=0.0, hi=1.0):
        return jax.random.uniform(self._next(), shape, jnp.bfloat16, lo, hi)
    def permutation(self, n):
        return jax.random.permutation(self._next(), n)


kernel_name = 'concat_heads__mha_block_cached__compressed_kv_cla__decode'

def setup_inputs():
    _rng = _Rng(jax.random.key(int.from_bytes(__import__("os").urandom(4), "little")))
    _w = (lambda a: (lambda t: t.astype(jnp.bfloat16) if jnp.issubdtype(t.dtype, jnp.floating) else t)(jnp.asarray(a)))
    def _A_setup():
        B, Sq, D = 4, 1, 576
        H, Sk, Dh = 32, 4096, 128
        return {
            "x": _w((lambda *s: _rng.normal(s) * 0.05)(B, Sq, D)),
            "k_cache": _w((lambda *s: _rng.normal(s) * 0.05)(B, H, Sk, Dh)),
            "v_cache": _w((lambda *s: _rng.normal(s) * 0.05)(B, H, Sk, Dh)),
            "wq": _w((lambda *s: _rng.normal(s) * 0.05)(D, H * Dh) * (D ** -0.5)),
            "wo": _w((lambda *s: _rng.normal(s) * 0.05)(H * Dh, D) * ((H * Dh) ** -0.5)),
        }
    _A_in = _A_setup()

    def _B_setup():
        B, H, Sq, Sk, D, M = 4, 32, 1, 4096, 128, 576
        Dc = 4 * D
        return {
            "x": _w((lambda *s: _rng.normal(s) * 0.05)(B, Sq, M)),
            "c_kv": _w((lambda *s: _rng.normal(s) * 0.05)(B, Sk, Dc)),
            "w_q": _w((lambda *s: _rng.normal(s) * 0.05)(M, H, D) * (M ** -0.5)),
            "w_uk": _w((lambda *s: _rng.normal(s) * 0.05)(Dc, H, D) * (Dc ** -0.5)),
            "w_uv": _w((lambda *s: _rng.normal(s) * 0.05)(Dc, H, D) * (Dc ** -0.5)),
            "w_o": _w((lambda *s: _rng.normal(s) * 0.05)(H, D, M) * ((H * D) ** -0.5)),
        }
    _B_in = _B_setup()

    return {
        "A_x": _A_in["x"],
        "A_k_cache": _A_in["k_cache"],
        "A_v_cache": _A_in["v_cache"],
        "A_wq": _A_in["wq"],
        "A_wo": _A_in["wo"],
        "B_x": _B_in["x"],
        "B_c_kv": _B_in["c_kv"],
        "B_w_q": _B_in["w_q"],
        "B_w_uk": _B_in["w_uk"],
        "B_w_uv": _B_in["w_uv"],
        "B_w_o": _B_in["w_o"],
    }

def reference(A_x, A_k_cache, A_v_cache, A_wq, A_wo, B_x, B_c_kv, B_w_q, B_w_uk, B_w_uv, B_w_o):
    def _A_ref(x, k_cache, v_cache, wq, wo):
        B, Sq, D = x.shape
        H, Dh = 32, 128
        q = (lambda x, *d: x.transpose(*d))((x @ wq).reshape(B, Sq, H, Dh), 0, 2, 1, 3)
        scores = jnp.einsum("bhqd,bhkd->bhqk", q, k_cache) * (Dh ** -0.5)
        p = _softmax(scores, axis=-1)
        o = jnp.einsum("bhqk,bhkd->bhqd", p, v_cache)
        return (lambda x, *d: x.transpose(*d))(o, 0, 2, 1, 3).reshape(B, Sq, H * Dh) @ wo

    def _B_ref(x, c_kv, w_q, w_uk, w_uv, w_o):
        B, Sq, M = x.shape[0], x.shape[1], x.shape[2]
        Sk = c_kv.shape[1]
        H, D = w_q.shape[1], w_q.shape[2]
        q = jnp.einsum("bqm,mhd->bhqd", x, w_q)
        k = jnp.einsum("bkc,chd->bhkd", c_kv, w_uk)
        v = jnp.einsum("bkc,chd->bhkd", c_kv, w_uv)
        scores = jnp.einsum("bhqd,bhkd->bhqk", q, k) * (D ** -0.5)
        off = Sk - Sq
        qi = jnp.arange(Sq)[:, None]
        kj = jnp.arange(Sk)[None, :]
        cmask = kj <= (qi + off)
        scores = jnp.where(cmask[None, None], scores, -1e9)
        p = _softmax(scores, axis=-1)
        ctx = jnp.einsum("bhqk,bhkd->bhqd", p, v)
        return jnp.einsum("bhqd,hdm->bqm", ctx, w_o)

    a = _A_ref(A_x, A_k_cache, A_v_cache, A_wq, A_wo)
    b = _B_ref(B_x, B_c_kv, B_w_q, B_w_uk, B_w_uv, B_w_o)
    return jnp.concatenate([a, b], axis=-1)
```

```python
import functools

import jax
import jax.numpy as jnp
from jax import lax
from jax.experimental import pallas as pl
from jax.experimental.pallas import tpu as pltpu

NB = 4
NH = 32
SK = 4096
DH = 128
DM = 576
DC = 512
NCH = DC // DH
NSTEP = NB * NH
NSLOTS = 8

F32 = jnp.float32
BF16 = jnp.bfloat16

S_XA, S_XB, S_WQ, S_WO, S_BWQ, S_WUK, S_WUV, S_BWO, S_CKV = 0, 1, 2, 3, 4, 5, 6, 7, 8
N_MISC = S_CKV + NB

T_CVT_Q = 10
T_CVT_UK = 11
T_HEAD0 = 12
T_ATTN0 = T_HEAD0 + NH
ATTN_STRIDE = 4
T_CVT_UV = T_ATTN0 + NB * ATTN_STRIDE
T_OUT0 = T_CVT_UV + 1

NT = (((1,), (1,)), ((), ()))
NN = (((1,), (0,)), ((), ()))


def _dot(a, b, dims):
    return lax.dot_general(a, b, dims, preferred_element_type=F32)


def _softmax_pv(s, v):
    m = jnp.max(s, axis=-1, keepdims=True)
    p = jnp.exp(s - m)
    l = jnp.sum(p, axis=-1, keepdims=True)
    o = _dot(p.astype(BF16), v, NN)
    return o / l


def _kernel(xa_hbm, k_hbm, v_hbm, wq_hbm, wo_hbm, xb_hbm, ckv_hbm, bwq_hbm,
            wuk_hbm, wuv_hbm, bwo_hbm,
            out_ref,
            kbuf, vbuf, xa_v, xb_v, wq_v, wo_v, ckv_v, bwq_v, wuk_v, wuv_v, bwo_v,
            w32a, w32b, qa_s, oa_s, outa_s, outb_s, qabs_s, ctxc_s,
            sem_k, sem_v, sem_m):
    scale = DH ** -0.5

    def slab(i):
        return (i % NB) * NH + i // NB

    def k_copy(i, slot):
        return pltpu.make_async_copy(k_hbm.at[slab(i)], kbuf.at[slot], sem_k.at[slot])

    def v_copy(i, slot):
        return pltpu.make_async_copy(v_hbm.at[slab(i)], vbuf.at[slot], sem_v.at[slot])

    def misc(src, dst, sid):
        return pltpu.make_async_copy(src, dst, sem_m.at[sid])

    cp_xa = misc(xa_hbm, xa_v, S_XA)
    cp_xb = misc(xb_hbm, xb_v, S_XB)
    cp_wq = misc(wq_hbm, wq_v, S_WQ)
    cp_wo = misc(wo_hbm, wo_v, S_WO)
    cp_bwq = misc(bwq_hbm, bwq_v, S_BWQ)
    cp_wuk = misc(wuk_hbm, wuk_v, S_WUK)
    cp_wuv = misc(wuv_hbm, wuv_v, S_WUV)
    cp_bwo = misc(bwo_hbm, bwo_v, S_BWO)

    def cp_ckv(b):
        return misc(ckv_hbm.at[b], ckv_v.at[b], S_CKV + b)

    cp_xa.start()
    cp_wq.start()
    for s in range(NSLOTS):
        k_copy(s, s).start()
        v_copy(s, s).start()
        if s == NB - 1:
            cp_wo.start()
    cp_xb.start()

    oa_s[...] = jnp.zeros(oa_s.shape, F32)
    outa_s[...] = jnp.zeros(outa_s.shape, F32)
    outb_s[...] = jnp.zeros(outb_s.shape, F32)

    cp_xa.wait()
    cp_wq.wait()
    qa = _dot(xa_v[...], wq_v[...], NN)
    for h in range(NH):
        qa_s[h] = qa[:, h * DH:(h + 1) * DH].astype(BF16)

    def convert(src, dst, rows):
        chunk = 1024
        def body(c, carry):
            r = pl.multiple_of(c * chunk, chunk)
            dst[pl.ds(r, chunk), :] = src[pl.ds(r, chunk), :].astype(F32)
            return carry
        lax.fori_loop(0, rows // chunk, body, 0)

    def step(i, carry):
        slot = i % NSLOTS
        h = i // NB
        b = i % NB

        k_copy(i, slot).wait()
        s = _dot(qa_s[h], kbuf[slot], NT) * scale
        v_copy(i, slot).wait()
        o = _softmax_pv(s, vbuf[slot])
        row = lax.broadcasted_iota(jnp.int32, (NB, DH), 0)
        oa = jnp.where(row == b, o, oa_s[...])
        oa_s[...] = oa

        @pl.when(i + NSLOTS < NSTEP)
        def _():
            k_copy(i + NSLOTS, slot).start()
            v_copy(i + NSLOTS, slot).start()

        @pl.when(b == NB - 1)
        def _():
            @pl.when(i == NB - 1)
            def _():
                cp_wo.wait()
            col = pl.multiple_of(h * DH, DH)
            outa_s[...] += _dot(oa.astype(BF16), wo_v[:, pl.ds(col, DH)], NT)

        @pl.when(i == 0)
        def _():
            cp_bwq.start()

        @pl.when(i == 1)
        def _():
            cp_wuk.start()

        for bb in range(NB):
            @pl.when(i == 2 + bb)
            def _():
                cp_ckv(bb).start()

        @pl.when(i == 2 + NB)
        def _():
            cp_wuv.start()

        @pl.when(i == 3 + NB)
        def _():
            cp_bwo.start()

        @pl.when(i == T_CVT_Q)
        def _():
            cp_xb.wait()
            cp_bwq.wait()
            convert(bwq_v, w32a, DM * NH)

        @pl.when(i == T_CVT_UK)
        def _():
            cp_wuk.wait()
            convert(wuk_v, w32b, DC * NH)

        @pl.when(jnp.logical_and(i >= T_HEAD0, i < T_HEAD0 + NH))
        def _():
            hh = i - T_HEAD0
            wq_h = w32a[pl.ds(hh, DM, stride=NH), :].astype(BF16)
            qb = _dot(xb_v[...], wq_h, NN).astype(BF16)
            wuk_h = w32b[pl.ds(hh, DC, stride=NH), :].astype(BF16)
            qabs = _dot(qb, wuk_h, NT)
            for j in range(NCH):
                qabs_s[j, pl.ds(hh, NB, stride=NH), :] = qabs[:, j * DH:(j + 1) * DH]

        for bb in range(NB):
            @pl.when(i == T_ATTN0 + bb * ATTN_STRIDE)
            def _():
                cp_ckv(bb).wait()
                q = jnp.concatenate(
                    [qabs_s[j, bb * NH:(bb + 1) * NH, :] for j in range(NCH)],
                    axis=1).astype(BF16)
                c = ckv_v[bb]
                sb = _dot(q, c, NT) * scale
                cc = _softmax_pv(sb, c)
                for j in range(NCH):
                    ctxc_s[j, bb * NH:(bb + 1) * NH, :] = cc[:, j * DH:(j + 1) * DH]

        @pl.when(i == T_CVT_UV)
        def _():
            cp_wuv.wait()
            cp_bwo.wait()
            convert(wuv_v, w32a, DC * NH)

        @pl.when(jnp.logical_and(i >= T_OUT0, i < T_OUT0 + NH))
        def _():
            hh = i - T_OUT0
            cc = jnp.concatenate(
                [ctxc_s[j, pl.ds(hh, NB, stride=NH), :] for j in range(NCH)],
                axis=1).astype(BF16)
            wuv_h = w32a[pl.ds(hh, DC, stride=NH), :].astype(BF16)
            ctx = _dot(cc, wuv_h, NN).astype(BF16)
            outb_s[...] += _dot(ctx, bwo_v[hh], NT)

        return carry

    lax.fori_loop(0, NSTEP, step, 0)

    out_ref[:, 0:DM] = outa_s[...].astype(out_ref.dtype)
    out_ref[:, DM:2 * DM] = outb_s[...].astype(out_ref.dtype)


@jax.jit
def pallas_concat_heads__mha_block_cached__compressed_kv_cla__decode_kernel(
    A_x: jax.Array,
    A_k_cache: jax.Array,
    A_v_cache: jax.Array,
    A_wq: jax.Array,
    A_wo: jax.Array,
    B_x: jax.Array,
    B_c_kv: jax.Array,
    B_w_q: jax.Array,
    B_w_uk: jax.Array,
    B_w_uv: jax.Array,
    B_w_o: jax.Array,
):
    xa = A_x.reshape(NB, DM)
    xb = B_x.reshape(NB, DM)
    k = A_k_cache.reshape(NSTEP, SK, DH)
    v = A_v_cache.reshape(NSTEP, SK, DH)
    wo_t = A_wo.T
    bwq = B_w_q.reshape(DM * NH, DH)
    wuk = B_w_uk.reshape(DC * NH, DH)
    wuv = B_w_uv.reshape(DC * NH, DH)
    bwo_t = B_w_o.transpose(0, 2, 1)

    any_spec = pl.BlockSpec(memory_space=pl.ANY)
    scratch = [
        pltpu.VMEM((NSLOTS, SK, DH), BF16),
        pltpu.VMEM((NSLOTS, SK, DH), BF16),
        pltpu.VMEM((NB, DM), BF16),
        pltpu.VMEM((NB, DM), BF16),
        pltpu.VMEM((DM, NH * DH), BF16),
        pltpu.VMEM((DM, NH * DH), BF16),
        pltpu.VMEM((NB, SK, DC), BF16),
        pltpu.VMEM((DM * NH, DH), BF16),
        pltpu.VMEM((DC * NH, DH), BF16),
        pltpu.VMEM((DC * NH, DH), BF16),
        pltpu.VMEM((NH, DM, DH), BF16),
        pltpu.VMEM((DM * NH, DH), F32),
        pltpu.VMEM((DC * NH, DH), F32),
        pltpu.VMEM((NH, NB, DH), BF16),
        pltpu.VMEM((NB, DH), F32),
        pltpu.VMEM((NB, DM), F32),
        pltpu.VMEM((NB, DM), F32),
        pltpu.VMEM((NCH, NB * NH, DH), F32),
        pltpu.VMEM((NCH, NB * NH, DH), F32),
        pltpu.SemaphoreType.DMA((NSLOTS,)),
        pltpu.SemaphoreType.DMA((NSLOTS,)),
        pltpu.SemaphoreType.DMA((N_MISC,)),
    ]
    out = pl.pallas_call(
        _kernel,
        out_shape=jax.ShapeDtypeStruct((NB, 2 * DM), BF16),
        in_specs=[any_spec] * 11,
        out_specs=pl.BlockSpec(memory_space=pltpu.VMEM),
        scratch_shapes=scratch,
        compiler_params=pltpu.CompilerParams(vmem_limit_bytes=112 * 1024 * 1024),
        name="fused_decode",
    )(xa, k, v, A_wq, wo_t, xb, B_c_kv, bwq, wuk, wuv, bwo_t)
    return out.reshape(NB, 1, 2 * DM)
```

```python
import jax
import jax.numpy as jnp
from jax import lax
from jax.experimental import pallas as pl
from jax.experimental.pallas import tpu as pltpu

NB = 4
NH = 32
SK = 4096
DH = 128
DM = 576
DC = 512
NCH = DC // DH
NSTEP = NB * NH
Z = NSTEP - 1

KV_CHUNK = 104
W_CHUNK = 104
C_CHUNK = 24
WIDE_COLS = ((0, 1536), (1536, 1536), (3072, 1024))
NW = 4
NC = 2
NG = 4
AHEAD = NG + 1
NSLOTS = AHEAD + 1
NZ = 4
TM, TL = 2048, 3072


def _chunks(lo, hi, c):
    return tuple((r, min(c, hi - r)) for r in range(lo, hi, c))


def _interleave(streams):
    out = []
    for j in range(max(len(s) for s in streams)):
        out += [s[j] for s in streams if j < len(s)]
    return out


_KV = _chunks(0, SK, KV_CHUNK)
assert len(_KV) % NG == 0
_GL = len(_KV) // NG
KV_GROUPS = tuple(_KV[g * _GL:(g + 1) * _GL] for g in range(NG))

F32 = jnp.float32
BF16 = jnp.bfloat16

S_XA, S_XB, S_WQ, S_WO, S_BWQ, S_WUK, S_WUV, S_BWO, S_CKV = range(9)
S_T0 = S_CKV + NB
S_T1 = S_T0 + 1
N_MISC = S_T1 + 1

T_CVT_Q = 6
T_CVT_UK = 7
T_HEAD0 = 8
T_ATTN0 = T_HEAD0 + NH
T_CVT_UV = T_ATTN0 + 2 * NB
T_OUT0 = T_CVT_UV + 1
assert T_OUT0 + NH <= NSTEP - NZ

NT = (((1,), (1,)), ((), ()))
NN = (((1,), (0,)), ((), ()))


def _dot(a, b, dims):
    return lax.dot_general(a, b, dims, preferred_element_type=F32)


def _softmax_num(s):
    m = jnp.max(s, axis=-1, keepdims=True)
    p = jnp.exp(s - m)
    l = jnp.sum(p, axis=-1, keepdims=True)
    return p.astype(BF16), l


def _kernel(xa_hbm, k_hbm, v_hbm, wq_hbm, wo_hbm, xb_hbm, ckv_hbm, bwq_hbm,
            wuk_hbm, wuv_hbm, bwo_hbm,
            out_ref,
            kbuf, vbuf, xa_v, xb_v, wq_v, wo_v, ckv_v, bwq_v, wuk_v, wuv_v, bwo_v,
            w32a, w32b, qa_s, oa_s, outa_s, outb_s, qabs_s, ctxc_s, pb_s, lb_s, p_s, l_s,
            sem_k, sem_v, sem_m):
    scale = DH ** -0.5

    def slab(i):
        return (i % NB) * NH + i // NB

    def k_start(i, r0, n):
        slot = i % NSLOTS
        pltpu.make_async_copy(k_hbm.at[slab(i), pl.ds(r0, n)], kbuf.at[slot, pl.ds(r0, n)],
                              sem_k.at[slot]).start(priority=0)

    def v_start(i, r0, n, sid=None):
        slot = i % NSLOTS
        sem = sem_v.at[slot] if sid is None else sem_m.at[sid]
        pltpu.make_async_copy(v_hbm.at[slab(i), pl.ds(r0, n)], vbuf.at[slot, pl.ds(r0, n)],
                              sem).start(priority=1)

    def kv_phase(p, groups, js):
        for j in js:
            for g in groups:
                r0, n = KV_GROUPS[g][j]
                k_start(p - g, r0, n)
                v_start(p - g, r0, n)

    def tail_list():
        kk = lambda i, g: [(k_start, (i, r, n)) for (r, n) in KV_GROUPS[g]]
        vv = lambda i, g: [(v_start, (i, r, n)) for (r, n) in KV_GROUPS[g]]
        x = (_interleave([kk(Z - 2, 3), vv(Z - 2, 3)])
             + _interleave([kk(Z - 1, 2), vv(Z - 1, 2), kk(Z - 1, 3), vv(Z - 1, 3)]))
        yk = kk(Z, 1) + kk(Z, 2) + kk(Z, 3)
        yv = []
        for lo, hi, sid in ((KV_GROUPS[1][0][0], TM, None), (TM, TL, S_T0), (TL, SK, S_T1)):
            yv += [(v_start, (Z, r, n, sid)) for (r, n) in _chunks(lo, hi, KV_CHUNK)]
        return x, yk, yv

    def issue(items):
        for fn, args in items:
            fn(*args)

    def wait_total(buf, sem):
        pltpu.make_async_copy(buf, buf, sem).wait()

    def k_wait(slot):
        wait_total(kbuf.at[slot], sem_k.at[slot])

    def v_wait(slot, lo=0, hi=SK, sid=None):
        wait_total(vbuf.at[slot, pl.ds(lo, hi - lo)],
                   sem_v.at[slot] if sid is None else sem_m.at[sid])

    def misc(src, dst, sid):
        return pltpu.make_async_copy(src, dst, sem_m.at[sid])

    def stream_rows(streams, rows, chunk):
        nfull, rem = rows // chunk, rows % chunk

        def one(r, n):
            for q, (src, dst, sid, off) in enumerate(streams):
                misc(src.at[pl.ds(off + r, n)], dst.at[pl.ds(off + r, n)],
                     sid).start(priority=q % 2)

        def body(j, c):
            one(pl.multiple_of(j * chunk, 8), chunk)
            return c

        lax.fori_loop(0, nfull, body, 0)
        if rem:
            one(nfull * chunk, rem)

    def stream_pair(src_a, dst_a, sid_a, src_b, dst_b, sid_b):
        rows = src_a.shape[0] // NW
        streams = []
        for m in range(NW):
            streams += [(src_a, dst_a, sid_a, m * rows), (src_b, dst_b, sid_b, m * rows)]
        stream_rows(streams, rows, W_CHUNK)

    def stream_wide_pair(src_a, dst_a, sid_a, src_b, dst_b, sid_b):
        rows = DM // NW

        def body(j, c):
            for (c0, n) in WIDE_COLS:
                for m in range(NW):
                    r = pl.multiple_of(m * rows + j * 8, 8)
                    misc(src_a.at[pl.ds(r, 8), pl.ds(c0, n)], dst_a.at[pl.ds(r, 8), pl.ds(c0, n)],
                         sid_a).start(priority=0)
                    misc(src_b.at[pl.ds(r, 8), pl.ds(c0, n)], dst_b.at[pl.ds(r, 8), pl.ds(c0, n)],
                         sid_b).start(priority=1)
            return c

        lax.fori_loop(0, rows // 8, body, 0)

    cp_xa = misc(xa_hbm, xa_v, S_XA)
    cp_xb = misc(xb_hbm, xb_v, S_XB)
    cp_xa.start()
    cp_xb.start()
    stream_wide_pair(wq_hbm, wq_v, S_WQ, wo_hbm, wo_v, S_WO)
    for p in range(AHEAD):
        kv_phase(p, range(min(p + 1, NG)), range(_GL))

    oa_s[...] = jnp.zeros(oa_s.shape, F32)
    outa_s[...] = jnp.zeros(outa_s.shape, F32)
    outb_s[...] = jnp.zeros(outb_s.shape, F32)

    cp_xa.wait()
    wait_total(wq_v, sem_m.at[S_WQ])
    qa = _dot(xa_v[...], wq_v[...], NN)
    for h in range(NH):
        qa_s[h] = qa[:, h * DH:(h + 1) * DH].astype(BF16)

    def to_f32(src, dst, rows):
        chunk = 1024

        def body(c, carry):
            r = pl.multiple_of(c * chunk, chunk)
            dst[pl.ds(r, chunk), :] = src[pl.ds(r, chunk), :].astype(F32)
            return carry

        lax.fori_loop(0, rows // chunk, body, 0)

    def out_proj(oa, h):
        col = pl.multiple_of(h * DH, DH)
        return _dot(oa.astype(BF16), wo_v[:, pl.ds(col, DH)], NT)

    tail_x, tail_yk, tail_yv = tail_list()

    def step(i, carry):
        slot = i % NSLOTS
        h = i // NB
        b = i % NB

        @pl.when(i + AHEAD < NSTEP)
        def _():
            kv_phase(i + AHEAD, range(NG), range(_GL // 2))

        @pl.when(i + AHEAD == NSTEP)
        def _():
            issue(tail_x)

        k_wait(slot)
        s = _dot(qa_s[h], kbuf[slot], NT) * scale
        p, l = _softmax_num(s)
        v_wait(slot)
        o = _dot(p, vbuf[slot], NN) / l
        row = lax.broadcasted_iota(jnp.int32, (NB, DH), 0)
        oa = jnp.where(row == b, o, oa_s[...])
        oa_s[...] = oa

        @pl.when(b == NB - 1)
        def _():
            @pl.when(i == NB - 1)
            def _():
                wait_total(wo_v, sem_m.at[S_WO])
            outa_s[...] += out_proj(oa, h)

        @pl.when(i + AHEAD < NSTEP)
        def _():
            kv_phase(i + AHEAD, range(NG), range(_GL // 2, _GL))

        @pl.when(i == 0)
        def _():
            stream_pair(bwq_hbm, bwq_v, S_BWQ, bwo_hbm, bwo_v, S_BWO)

        @pl.when(i == 1)
        def _():
            stream_pair(wuk_hbm, wuk_v, S_WUK, wuv_hbm, wuv_v, S_WUV)

        @pl.when(i == 2)
        def _():
            stream_rows([(ckv_hbm.at[bb], ckv_v.at[bb], S_CKV + bb, m * (SK // NC))
                         for m in range(NC) for bb in range(NB)], SK // NC, C_CHUNK)

        @pl.when(i == T_CVT_Q)
        def _():
            cp_xb.wait()
            wait_total(bwq_v, sem_m.at[S_BWQ])
            to_f32(bwq_v, w32a, DM * NH)

        @pl.when(i == T_CVT_UK)
        def _():
            wait_total(wuk_v, sem_m.at[S_WUK])
            to_f32(wuk_v, w32b, DC * NH)

        @pl.when(jnp.logical_and(i >= T_HEAD0, i < T_HEAD0 + NH))
        def _():
            hh = i - T_HEAD0
            wq_h = w32a[pl.ds(hh, DM, stride=NH), :].astype(BF16)
            qb = _dot(xb_v[...], wq_h, NN).astype(BF16)
            wuk_h = w32b[pl.ds(hh, DC, stride=NH), :].astype(BF16)
            qabs = _dot(qb, wuk_h, NT)
            for j in range(NCH):
                qabs_s[j, pl.ds(hh, NB, stride=NH), :] = qabs[:, j * DH:(j + 1) * DH]

        tb = i - T_ATTN0
        bb = tb // 2
        in_attn = jnp.logical_and(tb >= 0, tb < 2 * NB)

        @pl.when(jnp.logical_and(in_attn, tb % 2 == 0))
        def _():
            wait_total(ckv_v.at[bb], sem_m.at[S_CKV + bb])
            r0 = pl.multiple_of(bb * NH, NH)
            q = jnp.concatenate([qabs_s[j, pl.ds(r0, NH), :] for j in range(NCH)],
                                axis=1).astype(BF16)
            sb = _dot(q, ckv_v[bb], NT) * scale
            pb, lb = _softmax_num(sb)
            pb_s[...] = pb
            lb_s[...] = jnp.broadcast_to(lb, lb_s.shape)

        @pl.when(jnp.logical_and(in_attn, tb % 2 == 1))
        def _():
            r0 = pl.multiple_of(bb * NH, NH)
            cc = _dot(pb_s[...], ckv_v[bb], NN)
            lb = lb_s[...]
            for j in range(NCH):
                ctxc_s[j, pl.ds(r0, NH), :] = cc[:, j * DH:(j + 1) * DH] / lb

        @pl.when(i == T_CVT_UV)
        def _():
            wait_total(wuv_v, sem_m.at[S_WUV])
            wait_total(bwo_v, sem_m.at[S_BWO])
            to_f32(wuv_v, w32a, DC * NH)

        @pl.when(jnp.logical_and(i >= T_OUT0, i < T_OUT0 + NH))
        def _():
            hh = i - T_OUT0
            cc = jnp.concatenate([ctxc_s[j, pl.ds(hh, NB, stride=NH), :] for j in range(NCH)],
                                 axis=1).astype(BF16)
            wuv_h = w32a[pl.ds(hh, DC, stride=NH), :].astype(BF16)
            ctx = _dot(cc, wuv_h, NN).astype(BF16)
            r0 = pl.multiple_of(hh * DM, 8)
            outb_s[...] += _dot(ctx, bwo_v[pl.ds(r0, DM), :], NT)

        return carry

    lax.fori_loop(0, NSTEP - NZ, step, 0)

    def qk(i):
        slot = i % NSLOTS
        k_wait(slot)
        s = _dot(qa_s[i // NB], kbuf[slot], NT) * scale
        p, l = _softmax_num(s)
        p_s[i % NZ] = p
        l_s[i % NZ] = jnp.broadcast_to(l, (NB, DH))

    def pv(i, lo=0, hi=SK, sid=None):
        slot = i % NSLOTS
        v_wait(slot, lo, hi, sid)
        return _dot(p_s[i % NZ, :, lo:hi], vbuf[slot, lo:hi, :], NN)

    def keep_row(i, o, oa):
        row = lax.broadcasted_iota(jnp.int32, (NB, DH), 0)
        return jnp.where(row == i % NB, o / l_s[i % NZ], oa)

    oa = oa_s[...]
    issue(tail_yk)
    qk(Z - 3)
    qk(Z - 2)
    oa = keep_row(Z - 3, pv(Z - 3), oa)
    issue(tail_yv)
    qk(Z - 1)
    oa = keep_row(Z - 2, pv(Z - 2), oa)
    qk(Z)
    oa = keep_row(Z - 1, pv(Z - 1), oa)
    o = pv(Z, 0, TM)
    o = o + pv(Z, TM, TL, S_T0)
    o = o + pv(Z, TL, SK, S_T1)
    oa = keep_row(Z, o, oa)
    outa = outa_s[...] + out_proj(oa, NH - 1)

    out_ref[:, DM:2 * DM] = outb_s[...].astype(out_ref.dtype)
    out_ref[:, 0:DM] = outa.astype(out_ref.dtype)


@jax.jit
def pallas_concat_heads__mha_block_cached__compressed_kv_cla__decode_kernel(
    A_x: jax.Array,
    A_k_cache: jax.Array,
    A_v_cache: jax.Array,
    A_wq: jax.Array,
    A_wo: jax.Array,
    B_x: jax.Array,
    B_c_kv: jax.Array,
    B_w_q: jax.Array,
    B_w_uk: jax.Array,
    B_w_uv: jax.Array,
    B_w_o: jax.Array,
):
    xa = A_x.reshape(NB, DM)
    xb = B_x.reshape(NB, DM)
    k = A_k_cache.reshape(NSTEP, SK, DH)
    v = A_v_cache.reshape(NSTEP, SK, DH)
    wo_t = A_wo.T
    bwq = B_w_q.reshape(DM * NH, DH)
    wuk = B_w_uk.reshape(DC * NH, DH)
    wuv = B_w_uv.reshape(DC * NH, DH)
    bwo_t = B_w_o.transpose(0, 2, 1).reshape(NH * DM, DH)

    any_spec = pl.BlockSpec(memory_space=pl.ANY)
    scratch = [
        pltpu.VMEM((NSLOTS, SK, DH), BF16),
        pltpu.VMEM((NSLOTS, SK, DH), BF16),
        pltpu.VMEM((NB, DM), BF16),
        pltpu.VMEM((NB, DM), BF16),
        pltpu.VMEM((DM, NH * DH), BF16),
        pltpu.VMEM((DM, NH * DH), BF16),
        pltpu.VMEM((NB, SK, DC), BF16),
        pltpu.VMEM((DM * NH, DH), BF16),
        pltpu.VMEM((DC * NH, DH), BF16),
        pltpu.VMEM((DC * NH, DH), BF16),
        pltpu.VMEM((NH * DM, DH), BF16),
        pltpu.VMEM((DM * NH, DH), F32),
        pltpu.VMEM((DC * NH, DH), F32),
        pltpu.VMEM((NH, NB, DH), BF16),
        pltpu.VMEM((NB, DH), F32),
        pltpu.VMEM((NB, DM), F32),
        pltpu.VMEM((NB, DM), F32),
        pltpu.VMEM((NCH, NB * NH, DH), F32),
        pltpu.VMEM((NCH, NB * NH, DH), F32),
        pltpu.VMEM((NH, SK), BF16),
        pltpu.VMEM((NH, DH), F32),
        pltpu.VMEM((NZ, NB, SK), BF16),
        pltpu.VMEM((NZ, NB, DH), F32),
        pltpu.SemaphoreType.DMA((NSLOTS,)),
        pltpu.SemaphoreType.DMA((NSLOTS,)),
        pltpu.SemaphoreType.DMA((N_MISC,)),
    ]
    out = pl.pallas_call(
        _kernel,
        out_shape=jax.ShapeDtypeStruct((NB, 2 * DM), BF16),
        in_specs=[any_spec] * 11,
        out_specs=pl.BlockSpec(memory_space=pltpu.VMEM),
        scratch_shapes=scratch,
        compiler_params=pltpu.CompilerParams(
            vmem_limit_bytes=112 * 1024 * 1024,
            disable_bounds_checks=True,
            disable_semaphore_checks=True,
        ),
        name="fused_decode",
    )(xa, k, v, A_wq, wo_t, xb, B_c_kv, bwq, wuk, wuv, bwo_t)
    return out.reshape(NB, 1, 2 * DM)
```

```python
import jax
import jax.numpy as jnp
from jax import lax
from jax.experimental import pallas as pl
from jax.experimental.pallas import tpu as pltpu

NB = 4
NH = 32
SK = 4096
DH = 128
DM = 576
DC = 512
NCH = DC // DH
NSTEP = NB * NH
Z = NSTEP - 1

KV_CHUNK = 128
V_ROT = 6
W_CHUNK = 128
W_FIRST = 16
C_CHUNK = 32
WIDE_COLS = ((0, 2048), (2048, 2048))
NW = 4
NC = 2
NG = 4
AHEAD = NG + 1
NSLOTS = AHEAD + 1
NZ = 4
TM, TL = 2048, 3072


def _chunks(lo, hi, c):
    return tuple((r, min(c, hi - r)) for r in range(lo, hi, c))


def _interleave(streams):
    out = []
    for j in range(max(len(s) for s in streams)):
        out += [s[j] for s in streams if j < len(s)]
    return out


_KV = _chunks(0, SK, KV_CHUNK)
assert len(_KV) % NG == 0
_GL = len(_KV) // NG
KV_GROUPS = tuple(_KV[g * _GL:(g + 1) * _GL] for g in range(NG))

F32 = jnp.float32
BF16 = jnp.bfloat16

S_XA, S_XB, S_WQ, S_WO, S_BWQ, S_WUK, S_WUV, S_BWO, S_CKV = range(9)
S_T0 = S_CKV + NB
S_T1 = S_T0 + 1
N_MISC = S_T1 + 1

T_CVT_Q = 6
T_CVT_UK = 7
T_HEAD0 = 8
T_ATTN0 = T_HEAD0 + NH
T_CVT_UV = T_ATTN0 + 2 * NB
T_OUT0 = T_CVT_UV + 1
assert T_OUT0 + NH <= NSTEP - NZ

NT = (((1,), (1,)), ((), ()))
NN = (((1,), (0,)), ((), ()))


def _dot(a, b, dims):
    return lax.dot_general(a, b, dims, preferred_element_type=F32)


def _softmax_num(s):
    m = jnp.max(s, axis=-1, keepdims=True)
    p = jnp.exp(s - m)
    l = jnp.sum(p, axis=-1, keepdims=True)
    return p.astype(BF16), l


def _kernel(xa_hbm, k_hbm, v_hbm, wq_hbm, wo_hbm, xb_hbm, ckv_hbm, bwq_hbm,
            wuk_hbm, wuv_hbm, bwo_hbm,
            out_ref,
            kbuf, vbuf, xa_v, xb_v, wq_v, wo_v, ckv_v, bwq_v, wuk_v, wuv_v, bwo_v,
            w32a, w32b, qa_s, oa_s, outa_s, outb_s, qabs_s, ctxc_s, pb_s, lb_s, p_s, l_s,
            sem_k, sem_v, sem_m):
    scale = DH ** -0.5

    def slab(i):
        return (i % NB) * NH + i // NB

    def k_start(i, r0, n):
        slot = i % NSLOTS
        pltpu.make_async_copy(k_hbm.at[slab(i), pl.ds(r0, n)], kbuf.at[slot, pl.ds(r0, n)],
                              sem_k.at[slot]).start(priority=0)

    def v_start(i, r0, n, sid=None):
        slot = i % NSLOTS
        sem = sem_v.at[slot] if sid is None else sem_m.at[sid]
        pltpu.make_async_copy(v_hbm.at[slab(i), pl.ds(r0, n)], vbuf.at[slot, pl.ds(r0, n)],
                              sem).start(priority=1)

    def kv_phase(p, groups, js):
        for j in js:
            for g in groups:
                k_start(p - g, *KV_GROUPS[g][j])
                v_start(p - g, *KV_GROUPS[g][(j + V_ROT) % _GL])

    def tail_list():
        kk = lambda i, g: [(k_start, (i, r, n)) for (r, n) in KV_GROUPS[g]]
        vv = lambda i, g: [(v_start, (i, r, n)) for (r, n) in KV_GROUPS[g]]
        x = (_interleave([kk(Z - 2, 3), vv(Z - 2, 3)])
             + _interleave([kk(Z - 1, 2), vv(Z - 1, 2), kk(Z - 1, 3), vv(Z - 1, 3)]))
        yk = kk(Z, 1) + kk(Z, 2) + kk(Z, 3)
        yv = []
        for lo, hi, sid in ((KV_GROUPS[1][0][0], TM, None), (TM, TL, S_T0), (TL, SK, S_T1)):
            yv += [(v_start, (Z, r, n, sid)) for (r, n) in _chunks(lo, hi, KV_CHUNK)]
        return x, yk, yv

    def issue(items):
        for fn, args in items:
            fn(*args)

    def wait_total(buf, sem):
        pltpu.make_async_copy(buf, buf, sem).wait()

    def k_wait(slot):
        wait_total(kbuf.at[slot], sem_k.at[slot])

    def v_wait(slot, lo=0, hi=SK, sid=None):
        wait_total(vbuf.at[slot, pl.ds(lo, hi - lo)],
                   sem_v.at[slot] if sid is None else sem_m.at[sid])

    def misc(src, dst, sid):
        return pltpu.make_async_copy(src, dst, sem_m.at[sid])

    def stream_rows(arrays, chunk, first, ns):
        total = arrays[0][0].shape[0]
        nfull = (total - first) // chunk
        per = nfull // ns

        def one(r, n):
            for q, (src, dst, sid) in enumerate(arrays):
                misc(src.at[pl.ds(r, n)], dst.at[pl.ds(r, n)], sid).start(priority=q % 2)

        def body(j, c):
            for m in range(ns):
                one(pl.multiple_of(first + (m * per + j) * chunk, 8), chunk)
            return c

        if first:
            one(0, first)
        lax.fori_loop(0, per, body, 0)
        for (r, n) in _chunks(first + ns * per * chunk, total, chunk):
            one(r, n)

    def stream_wide_pair(src_a, dst_a, sid_a, src_b, dst_b, sid_b):
        rows = DM // NW

        def body(j, c):
            for (c0, n) in WIDE_COLS:
                for m in range(NW):
                    r = pl.multiple_of(m * rows + j * 8, 8)
                    misc(src_a.at[pl.ds(r, 8), pl.ds(c0, n)], dst_a.at[pl.ds(r, 8), pl.ds(c0, n)],
                         sid_a).start(priority=0)
                    misc(src_b.at[pl.ds(r, 8), pl.ds(c0, n)], dst_b.at[pl.ds(r, 8), pl.ds(c0, n)],
                         sid_b).start(priority=1)
            return c

        lax.fori_loop(0, rows // 8, body, 0)

    cp_xa = misc(xa_hbm, xa_v, S_XA)
    cp_xb = misc(xb_hbm, xb_v, S_XB)
    cp_xa.start()
    cp_xb.start()
    stream_wide_pair(wq_hbm, wq_v, S_WQ, wo_hbm, wo_v, S_WO)
    for p in range(AHEAD):
        kv_phase(p, range(min(p + 1, NG)), range(_GL))

    oa_s[...] = jnp.zeros(oa_s.shape, F32)
    outa_s[...] = jnp.zeros(outa_s.shape, F32)
    outb_s[...] = jnp.zeros(outb_s.shape, F32)

    cp_xa.wait()
    wait_total(wq_v, sem_m.at[S_WQ])
    qa = _dot(xa_v[...], wq_v[...], NN)
    for h in range(NH):
        qa_s[h] = qa[:, h * DH:(h + 1) * DH].astype(BF16)

    def to_f32(src, dst, rows):
        chunk = 1024

        def body(c, carry):
            r = pl.multiple_of(c * chunk, chunk)
            dst[pl.ds(r, chunk), :] = src[pl.ds(r, chunk), :].astype(F32)
            return carry

        lax.fori_loop(0, rows // chunk, body, 0)

    def out_proj(oa, h):
        col = pl.multiple_of(h * DH, DH)
        return _dot(oa.astype(BF16), wo_v[:, pl.ds(col, DH)], NT)

    tail_x, tail_yk, tail_yv = tail_list()

    def step(i, carry):
        slot = i % NSLOTS
        h = i // NB
        b = i % NB

        @pl.when(i + AHEAD < NSTEP)
        def _():
            kv_phase(i + AHEAD, range(NG), range(_GL // 2))

        @pl.when(i + AHEAD == NSTEP)
        def _():
            issue(tail_x)

        k_wait(slot)
        s = _dot(qa_s[h], kbuf[slot], NT) * scale
        p, l = _softmax_num(s)
        v_wait(slot)
        o = _dot(p, vbuf[slot], NN) / l
        row = lax.broadcasted_iota(jnp.int32, (NB, DH), 0)
        oa = jnp.where(row == b, o, oa_s[...])
        oa_s[...] = oa

        @pl.when(b == NB - 1)
        def _():
            @pl.when(i == NB - 1)
            def _():
                wait_total(wo_v, sem_m.at[S_WO])
            outa_s[...] += out_proj(oa, h)

        @pl.when(i + AHEAD < NSTEP)
        def _():
            kv_phase(i + AHEAD, range(NG), range(_GL // 2, _GL))

        @pl.when(i == 0)
        def _():
            stream_rows([(bwq_hbm, bwq_v, S_BWQ), (bwo_hbm, bwo_v, S_BWO)], W_CHUNK, W_FIRST, NW)

        @pl.when(i == 1)
        def _():
            stream_rows([(wuk_hbm, wuk_v, S_WUK), (wuv_hbm, wuv_v, S_WUV)], W_CHUNK, W_FIRST, NW)

        @pl.when(i == 2)
        def _():
            stream_rows([(ckv_hbm.at[bb], ckv_v.at[bb], S_CKV + bb) for bb in range(NB)],
                        C_CHUNK, 0, NC)

        @pl.when(i == T_CVT_Q)
        def _():
            cp_xb.wait()
            wait_total(bwq_v, sem_m.at[S_BWQ])
            to_f32(bwq_v, w32a, DM * NH)

        @pl.when(i == T_CVT_UK)
        def _():
            wait_total(wuk_v, sem_m.at[S_WUK])
            to_f32(wuk_v, w32b, DC * NH)

        @pl.when(jnp.logical_and(i >= T_HEAD0, i < T_HEAD0 + NH))
        def _():
            hh = i - T_HEAD0
            wq_h = w32a[pl.ds(hh, DM, stride=NH), :].astype(BF16)
            qb = _dot(xb_v[...], wq_h, NN).astype(BF16)
            wuk_h = w32b[pl.ds(hh, DC, stride=NH), :].astype(BF16)
            qabs = _dot(qb, wuk_h, NT)
            for j in range(NCH):
                qabs_s[j, pl.ds(hh, NB, stride=NH), :] = qabs[:, j * DH:(j + 1) * DH]

        tb = i - T_ATTN0
        bb = tb // 2
        in_attn = jnp.logical_and(tb >= 0, tb < 2 * NB)

        @pl.when(jnp.logical_and(in_attn, tb % 2 == 0))
        def _():
            wait_total(ckv_v.at[bb], sem_m.at[S_CKV + bb])
            r0 = pl.multiple_of(bb * NH, NH)
            q = jnp.concatenate([qabs_s[j, pl.ds(r0, NH), :] for j in range(NCH)],
                                axis=1).astype(BF16)
            sb = _dot(q, ckv_v[bb], NT) * scale
            pb, lb = _softmax_num(sb)
            pb_s[...] = pb
            lb_s[...] = jnp.broadcast_to(lb, lb_s.shape)

        @pl.when(jnp.logical_and(in_attn, tb % 2 == 1))
        def _():
            r0 = pl.multiple_of(bb * NH, NH)
            cc = _dot(pb_s[...], ckv_v[bb], NN)
            lb = lb_s[...]
            for j in range(NCH):
                ctxc_s[j, pl.ds(r0, NH), :] = cc[:, j * DH:(j + 1) * DH] / lb

        @pl.when(i == T_CVT_UV)
        def _():
            wait_total(wuv_v, sem_m.at[S_WUV])
            wait_total(bwo_v, sem_m.at[S_BWO])
            to_f32(wuv_v, w32a, DC * NH)

        @pl.when(jnp.logical_and(i >= T_OUT0, i < T_OUT0 + NH))
        def _():
            hh = i - T_OUT0
            cc = jnp.concatenate([ctxc_s[j, pl.ds(hh, NB, stride=NH), :] for j in range(NCH)],
                                 axis=1).astype(BF16)
            wuv_h = w32a[pl.ds(hh, DC, stride=NH), :].astype(BF16)
            ctx = _dot(cc, wuv_h, NN).astype(BF16)
            r0 = pl.multiple_of(hh * DM, 8)
            outb_s[...] += _dot(ctx, bwo_v[pl.ds(r0, DM), :], NT)

        return carry

    lax.fori_loop(0, NSTEP - NZ, step, 0)

    def qk(i):
        slot = i % NSLOTS
        k_wait(slot)
        s = _dot(qa_s[i // NB], kbuf[slot], NT) * scale
        p, l = _softmax_num(s)
        p_s[i % NZ] = p
        l_s[i % NZ] = jnp.broadcast_to(l, (NB, DH))

    def pv(i, lo=0, hi=SK, sid=None):
        slot = i % NSLOTS
        v_wait(slot, lo, hi, sid)
        return _dot(p_s[i % NZ, :, lo:hi], vbuf[slot, lo:hi, :], NN)

    def keep_row(i, o, oa):
        row = lax.broadcasted_iota(jnp.int32, (NB, DH), 0)
        return jnp.where(row == i % NB, o / l_s[i % NZ], oa)

    oa = oa_s[...]
    issue(tail_yk)
    qk(Z - 3)
    qk(Z - 2)
    issue(tail_yv)
    qk(Z - 1)
    oa = keep_row(Z - 3, pv(Z - 3), oa)
    qk(Z)
    oa = keep_row(Z - 2, pv(Z - 2), oa)
    oa = keep_row(Z - 1, pv(Z - 1), oa)
    o = pv(Z, 0, TM)
    o = o + pv(Z, TM, TL, S_T0)
    o = o + pv(Z, TL, SK, S_T1)
    oa = keep_row(Z, o, oa)
    outa = outa_s[...] + out_proj(oa, NH - 1)

    out_ref[:, DM:2 * DM] = outb_s[...].astype(out_ref.dtype)
    out_ref[:, 0:DM] = outa.astype(out_ref.dtype)


@jax.jit
def pallas_concat_heads__mha_block_cached__compressed_kv_cla__decode_kernel(
    A_x: jax.Array,
    A_k_cache: jax.Array,
    A_v_cache: jax.Array,
    A_wq: jax.Array,
    A_wo: jax.Array,
    B_x: jax.Array,
    B_c_kv: jax.Array,
    B_w_q: jax.Array,
    B_w_uk: jax.Array,
    B_w_uv: jax.Array,
    B_w_o: jax.Array,
):
    xa = A_x.reshape(NB, DM)
    xb = B_x.reshape(NB, DM)
    k = A_k_cache.reshape(NSTEP, SK, DH)
    v = A_v_cache.reshape(NSTEP, SK, DH)
    wo_t = A_wo.T
    bwq = B_w_q.reshape(DM * NH, DH)
    wuk = B_w_uk.reshape(DC * NH, DH)
    wuv = B_w_uv.reshape(DC * NH, DH)
    bwo_t = B_w_o.transpose(0, 2, 1).reshape(NH * DM, DH)

    any_spec = pl.BlockSpec(memory_space=pl.ANY)
    scratch = [
        pltpu.VMEM((NSLOTS, SK, DH), BF16),
        pltpu.VMEM((NSLOTS, SK, DH), BF16),
        pltpu.VMEM((NB, DM), BF16),
        pltpu.VMEM((NB, DM), BF16),
        pltpu.VMEM((DM, NH * DH), BF16),
        pltpu.VMEM((DM, NH * DH), BF16),
        pltpu.VMEM((NB, SK, DC), BF16),
        pltpu.VMEM((DM * NH, DH), BF16),
        pltpu.VMEM((DC * NH, DH), BF16),
        pltpu.VMEM((DC * NH, DH), BF16),
        pltpu.VMEM((NH * DM, DH), BF16),
        pltpu.VMEM((DM * NH, DH), F32),
        pltpu.VMEM((DC * NH, DH), F32),
        pltpu.VMEM((NH, NB, DH), BF16),
        pltpu.VMEM((NB, DH), F32),
        pltpu.VMEM((NB, DM), F32),
        pltpu.VMEM((NB, DM), F32),
        pltpu.VMEM((NCH, NB * NH, DH), F32),
        pltpu.VMEM((NCH, NB * NH, DH), F32),
        pltpu.VMEM((NH, SK), BF16),
        pltpu.VMEM((NH, DH), F32),
        pltpu.VMEM((NZ, NB, SK), BF16),
        pltpu.VMEM((NZ, NB, DH), F32),
        pltpu.SemaphoreType.DMA((NSLOTS,)),
        pltpu.SemaphoreType.DMA((NSLOTS,)),
        pltpu.SemaphoreType.DMA((N_MISC,)),
    ]
    out = pl.pallas_call(
        _kernel,
        out_shape=jax.ShapeDtypeStruct((NB, 2 * DM), BF16),
        in_specs=[any_spec] * 11,
        out_specs=pl.BlockSpec(memory_space=pltpu.VMEM),
        scratch_shapes=scratch,
        compiler_params=pltpu.CompilerParams(
            vmem_limit_bytes=112 * 1024 * 1024,
            disable_bounds_checks=True,
            disable_semaphore_checks=True,
        ),
        name="fused_decode",
    )(xa, k, v, A_wq, wo_t, xb, B_c_kv, bwq, wuk, wuv, bwo_t)
    return out.reshape(NB, 1, 2 * DM)
```
